```python
import os as _os
_os.environ.setdefault("JAX_PLATFORMS", "cpu")
import jax
import jax.numpy as jnp

def _softmax(x, axis=-1):
    return jax.nn.softmax(x, axis=axis)
def _gelu(x):
    return jax.nn.gelu(x, approximate=True)
def _silu(x):
    return jax.nn.silu(x)
def _sigmoid(x):
    return jax.nn.sigmoid(x)
def _layernorm(x, axis=-1, eps=1e-5):
    m = jnp.mean(x, axis=axis, keepdims=True)
    v = jnp.var(x, axis=axis, keepdims=True)
    return (x - m) / jnp.sqrt(v + eps)
def _scatter_add(tgt, idx, src, axis=0):
    return tgt.at[idx].add(src)
def _segment_sum(src, seg, n):
    return jax.ops.segment_sum(src, seg, n)
class _Rng:
    def __init__(self, key):
        self._k = key
    def _next(self):
        self._k, sub = jax.random.split(self._k)
        return sub
    def normal(self, shape):
        return jax.random.normal(self._next(), shape, dtype=jnp.bfloat16)
    def randint(self, lo, hi, shape):
        return jax.random.randint(self._next(), shape, lo, hi, dtype=jnp.int32)
    def uniform(self, shape, lo=0.0, hi=1.0):
        return jax.random.uniform(self._next(), shape, jnp.bfloat16, lo, hi)
    def permutation(self, n):
        return jax.random.permutation(self._next(), n)


kernel_name = 'concat_heads__mha_block_cached__mha_block_cached__near_ridge'

def setup_inputs():
    _rng = _Rng(jax.random.key(int.from_bytes(__import__("os").urandom(4), "little")))
    _w = (lambda a: (lambda t: t.astype(jnp.bfloat16) if jnp.issubdtype(t.dtype, jnp.floating) else t)(jnp.asarray(a)))
    def _A_setup():
        B, Sq, D = 8, 160, 512
        H, Sk, Dh = 32, 512, 128
        return {
            "x": _w((lambda *s: _rng.normal(s) * 0.8)(B, Sq, D)),
            "k_cache": _w((lambda *s: _rng.normal(s) * 0.8)(B, H, Sk, Dh)),
            "v_cache": _w((lambda *s: _rng.normal(s) * 0.05)(B, H, Sk, Dh)),
            "wq": _w((lambda *s: _rng.normal(s) * 0.8)(D, H * Dh) * (D ** -0.5)),
            "wo": _w((lambda *s: _rng.normal(s) * 0.05)(H * Dh, D) * ((H * Dh) ** -0.5)),
        }
    _A_in = _A_setup()

    def _B_setup():
        B, Sq, D = 8, 160, 512
        H, Sk, Dh = 32, 512, 128
        return {
            "x": _w((lambda *s: _rng.normal(s) * 0.8)(B, Sq, D)),
            "k_cache": _w((lambda *s: _rng.normal(s) * 0.8)(B, H, Sk, Dh)),
            "v_cache": _w((lambda *s: _rng.normal(s) * 0.05)(B, H, Sk, Dh)),
            "wq": _w((lambda *s: _rng.normal(s) * 0.8)(D, H * Dh) * (D ** -0.5)),
            "wo": _w((lambda *s: _rng.normal(s) * 0.05)(H * Dh, D) * ((H * Dh) ** -0.5)),
        }
    _B_in = _B_setup()

    return {
        "A_x": _A_in["x"],
        "A_k_cache": _A_in["k_cache"],
        "A_v_cache": _A_in["v_cache"],
        "A_wq": _A_in["wq"],
        "A_wo": _A_in["wo"],
        "B_x": _B_in["x"],
        "B_k_cache": _B_in["k_cache"],
        "B_v_cache": _B_in["v_cache"],
        "B_wq": _B_in["wq"],
        "B_wo": _B_in["wo"],
    }

def reference(A_x, A_k_cache, A_v_cache, A_wq, A_wo, B_x, B_k_cache, B_v_cache, B_wq, B_wo):
    def _A_ref(x, k_cache, v_cache, wq, wo):
        B, Sq, D = x.shape
        H, Dh = 32, 128
        q = (lambda x, *d: x.transpose(*d))((x @ wq).reshape(B, Sq, H, Dh), 0, 2, 1, 3)
        scores = jnp.einsum("bhqd,bhkd->bhqk", q, k_cache) * (Dh ** -0.5)
        p = _softmax(scores, axis=-1)
        o = jnp.einsum("bhqk,bhkd->bhqd", p, v_cache)
        return (lambda x, *d: x.transpose(*d))(o, 0, 2, 1, 3).reshape(B, Sq, H * Dh) @ wo

    def _B_ref(x, k_cache, v_cache, wq, wo):
        B, Sq, D = x.shape
        H, Dh = 32, 128
        q = (lambda x, *d: x.transpose(*d))((x @ wq).reshape(B, Sq, H, Dh), 0, 2, 1, 3)
        scores = jnp.einsum("bhqd,bhkd->bhqk", q, k_cache) * (Dh ** -0.5)
        p = _softmax(scores, axis=-1)
        o = jnp.einsum("bhqk,bhkd->bhqd", p, v_cache)
        return (lambda x, *d: x.transpose(*d))(o, 0, 2, 1, 3).reshape(B, Sq, H * Dh) @ wo

    a = _A_ref(A_x, A_k_cache, A_v_cache, A_wq, A_wo)
    b = _B_ref(B_x, B_k_cache, B_v_cache, B_wq, B_wo)
    return jnp.concatenate([a, b], axis=-1)
```

```python
import jax
import jax.numpy as jnp
import jax.experimental.pallas as pl
import jax.experimental.pallas.tpu as pltpu

HG = 4


def _attn_group(x, wq_ref, k_ref, v_ref, wo_ref, scale):
    q = jnp.dot(x, wq_ref[...], preferred_element_type=jnp.float32)
    q = (q * scale).astype(jnp.bfloat16)
    outs = []
    for h in range(HG):
        qh = q[:, h * 128:(h + 1) * 128]
        s = jax.lax.dot_general(qh, k_ref[0, h], (((1,), (1,)), ((), ())),
                                preferred_element_type=jnp.float32)
        m = jnp.max(s, axis=-1, keepdims=True)
        p = jnp.exp(s - m)
        l = jnp.sum(p, axis=-1, keepdims=True)
        o = jnp.dot(p.astype(jnp.bfloat16), v_ref[0, h], preferred_element_type=jnp.float32)
        outs.append((o / l).astype(jnp.bfloat16))
    o = jnp.concatenate(outs, axis=-1)
    return jnp.dot(o, wo_ref[...], preferred_element_type=jnp.float32)


def _kernel(ax, ak, av, awq, awo, bx, bk, bv, bwq, bwo, o_ref, acc):
    g = pl.program_id(0)
    b = pl.program_id(1)
    ng = pl.num_programs(0)
    scale = 128 ** -0.5
    ra = _attn_group(ax[b], awq, ak, av, awo, scale)
    rb = _attn_group(bx[b], bwq, bk, bv, bwo, scale)

    @pl.when(g == 0)
    def _():
        acc[b, :, 0:512] = ra
        acc[b, :, 512:1024] = rb

    @pl.when(g > 0)
    def _():
        acc[b, :, 0:512] += ra
        acc[b, :, 512:1024] += rb

    @pl.when(g == ng - 1)
    def _():
        o_ref[0] = acc[b].astype(o_ref.dtype)


@jax.jit
def pallas_concat_heads__mha_block_cached__mha_block_cached__near_ridge_kernel(
    A_x: jax.Array,
    A_k_cache: jax.Array,
    A_v_cache: jax.Array,
    A_wq: jax.Array,
    A_wo: jax.Array,
    B_x: jax.Array,
    B_k_cache: jax.Array,
    B_v_cache: jax.Array,
    B_wq: jax.Array,
    B_wo: jax.Array,
):
    B, Sq, D = A_x.shape
    _, H, Sk, Dh = A_k_cache.shape
    ng = H // HG
    x_spec = pl.BlockSpec((B, Sq, D), lambda g, b: (0, 0, 0))
    kv_spec = pl.BlockSpec((1, HG, Sk, Dh), lambda g, b: (b, g, 0, 0))
    wq_spec = pl.BlockSpec((D, HG * Dh), lambda g, b: (0, g))
    wo_spec = pl.BlockSpec((HG * Dh, D), lambda g, b: (g, 0))
    specs = [x_spec, kv_spec, kv_spec, wq_spec, wo_spec]
    out_spec = pl.BlockSpec((1, Sq, 2 * D), lambda g, b: (jnp.where(g == ng - 1, b, 0), 0, 0))
    return pl.pallas_call(
        _kernel,
        grid=(ng, B),
        in_specs=specs + specs,
        out_specs=out_spec,
        out_shape=jax.ShapeDtypeStruct((B, Sq, 2 * D), jnp.bfloat16),
        scratch_shapes=[pltpu.VMEM((B, Sq, 2 * D), jnp.float32)],
        compiler_params=pltpu.CompilerParams(
            dimension_semantics=("arbitrary", "arbitrary"),
            vmem_limit_bytes=100 * 1024 * 1024),
    )(A_x, A_k_cache, A_v_cache, A_wq, A_wo, B_x, B_k_cache, B_v_cache, B_wq, B_wo)
```

```python
import jax
import jax.numpy as jnp
import jax.experimental.pallas as pl
import jax.experimental.pallas.tpu as pltpu

HG = 4
NB = 4
RING = 4
LAG = 2
DH = 128


def _qk(qh, kh):
    return jax.lax.dot_general(qh, kh, (((1,), (1,)), ((), ())),
                               preferred_element_type=jnp.float32)


def _softmax_pv(s, vh):
    m = jnp.max(s, axis=-1, keepdims=True)
    p = jnp.exp(s - m)
    l = jnp.sum(p, axis=-1, keepdims=True)
    o = jnp.dot(p.astype(jnp.bfloat16), vh, preferred_element_type=jnp.float32)
    r = pl.reciprocal(l, approx=True)
    r = r * (2.0 - l * r)
    return (o * r).astype(jnp.bfloat16)


def _kernel(ax, ak, av, awq, awo, bx, bk, bv, bwq, bwo, o_ref,
            acc, kvbuf, xbuf, wqbuf, wobuf, qbuf, kvsem, xsem, wsem):
    scale = DH ** -0.5
    t = pl.program_id(0)
    total = pl.num_programs(0)
    ng = qbuf.shape[1]
    nj = total // ng
    sq = acc.shape[1]
    d_model = xbuf.shape[2]
    g = t // nj
    j = t % nj
    kv_hbm = (ak, av, bk, bv)
    x_hbm = (ax, bx)
    wq_hbm = (awq, bwq)
    wo_hbm = (awo, bwo)
    w = HG * DH

    def kv_copy(tt, i):
        tj = tt % nj
        tg = tt // nj
        st = tt % RING
        return pltpu.make_async_copy(
            kv_hbm[i].at[pl.ds(tj * NB, NB), pl.ds(tg * HG, HG)],
            kvbuf.at[st, i], kvsem.at[st, i])

    def x_copy(br):
        return pltpu.make_async_copy(x_hbm[br], xbuf.at[br], xsem.at[br])

    def wq_copy(br, gg):
        return pltpu.make_async_copy(
            wq_hbm[br].at[:, pl.ds(gg * w, w)], wqbuf.at[br, gg], wsem.at[0, br, gg])

    def wo_copy(br, gg):
        return pltpu.make_async_copy(
            wo_hbm[br].at[pl.ds(gg * w, w), :], wobuf.at[br, gg], wsem.at[1, br, gg])

    @pl.when(t == 0)
    def _():
        x_copy(0).start()
        wq_copy(0, 0).start()
        acc[...] = jnp.zeros(acc.shape, acc.dtype)
        x_copy(0).wait()
        x_copy(1).start()
        wq_copy(1, 0).start()
        wq_copy(0, 1).start()
        wq_copy(1, 1).start()

        def body(gg, carry):
            for br in range(2):
                if br == 1:
                    @pl.when(gg == 0)
                    def _():
                        x_copy(1).wait()
                wq_copy(br, gg).wait()
                if br == 1:
                    @pl.when(gg == 0)
                    def _():
                        for g2 in range(2, ng):
                            wq_copy(0, g2).start()
                            wq_copy(1, g2).start()
                if br == 0:
                    @pl.when(jnp.logical_and(gg >= LAG, gg - LAG < RING - 1))
                    def _():
                        for i in range(4):
                            kv_copy(gg - LAG, i).start()
                else:
                    @pl.when(gg >= LAG)
                    def _():
                        wo_copy(0, gg - LAG).start()
                        wo_copy(1, gg - LAG).start()
                q = jnp.dot(xbuf[br], wqbuf[br, gg], preferred_element_type=jnp.float32)
                qbuf[br, gg] = (q * scale).astype(jnp.bfloat16)
            return carry

        jax.lax.fori_loop(0, ng, body, 0)
        for d in range(ng - LAG, RING - 1):
            for i in range(4):
                kv_copy(d, i).start()
        for gg in range(ng - LAG, ng):
            wo_copy(0, gg).start()
            wo_copy(1, gg).start()

    @pl.when(t + RING - 1 < total)
    def _():
        for i in range(4):
            kv_copy(t + RING - 1, i).start()

    @pl.when(j == 0)
    def _():
        wo_copy(0, g).wait()
        wo_copy(1, g).wait()

    for i in range(4):
        kv_copy(t, i).wait()
    cur = t % RING

    units = [(s, br, h) for s in range(NB) for br in range(2) for h in range(HG)]
    n = len(units)
    scores = {}

    def issue(i):
        s, br, h = units[i]
        r0 = pl.multiple_of((j * NB + s) * sq, 32)
        qh = qbuf[br, g, pl.ds(r0, sq), h * DH:(h + 1) * DH]
        scores[i] = _qk(qh, kvbuf[cur, 2 * br, s, h])

    issue(0)
    outs = []
    for i in range(n):
        if i + 1 < n:
            issue(i + 1)
        s, br, h = units[i]
        outs.append(_softmax_pv(scores.pop(i), kvbuf[cur, 2 * br + 1, s, h]))
        if h == HG - 1:
            b = j * NB + s
            o = jnp.concatenate(outs, axis=-1)
            outs = []
            acc[b, :, br * d_model:(br + 1) * d_model] += jnp.dot(
                o, wobuf[br, g], preferred_element_type=jnp.float32)

    @pl.when(g == ng - 1)
    def _():
        o_ref[...] = acc[pl.ds(j * NB, NB)].astype(o_ref.dtype)


@jax.jit
def pallas_concat_heads__mha_block_cached__mha_block_cached__near_ridge_kernel(
    A_x: jax.Array,
    A_k_cache: jax.Array,
    A_v_cache: jax.Array,
    A_wq: jax.Array,
    A_wo: jax.Array,
    B_x: jax.Array,
    B_k_cache: jax.Array,
    B_v_cache: jax.Array,
    B_wq: jax.Array,
    B_wo: jax.Array,
):
    B, Sq, D = A_x.shape
    _, H, Sk, Dh = A_k_cache.shape
    ng = H // HG
    nj = B // NB
    anyspec = pl.BlockSpec(memory_space=pl.ANY)
    out_spec = pl.BlockSpec(
        (NB, Sq, 2 * D), lambda t: (jnp.maximum(t - (ng - 1) * nj, 0), 0, 0))
    return pl.pallas_call(
        _kernel,
        grid=(ng * nj,),
        in_specs=[anyspec] * 10,
        out_specs=out_spec,
        out_shape=jax.ShapeDtypeStruct((B, Sq, 2 * D), jnp.bfloat16),
        scratch_shapes=[
            pltpu.VMEM((B, Sq, 2 * D), jnp.float32),
            pltpu.VMEM((RING, 4, NB, HG, Sk, Dh), jnp.bfloat16),
            pltpu.VMEM((2, B * Sq, D), jnp.bfloat16),
            pltpu.VMEM((2, ng, D, HG * Dh), jnp.bfloat16),
            pltpu.VMEM((2, ng, HG * Dh, D), jnp.bfloat16),
            pltpu.VMEM((2, ng, B * Sq, HG * Dh), jnp.bfloat16),
            pltpu.SemaphoreType.DMA((RING, 4)),
            pltpu.SemaphoreType.DMA((2,)),
            pltpu.SemaphoreType.DMA((2, 2, ng)),
        ],
        compiler_params=pltpu.CompilerParams(
            dimension_semantics=("arbitrary",),
            disable_bounds_checks=True,
            vmem_limit_bytes=120 * 1024 * 1024),
    )(A_x.reshape(B * Sq, D), A_k_cache, A_v_cache, A_wq, A_wo,
      B_x.reshape(B * Sq, D), B_k_cache, B_v_cache, B_wq, B_wo)
```

```python
import jax
import jax.numpy as jnp
import jax.experimental.pallas as pl
import jax.experimental.pallas.tpu as pltpu

HG = 4
NB = 4
RING = 4
LAG = 1
DH = 128


def _qk(qh, kh):
    return jax.lax.dot_general(qh, kh, (((1,), (1,)), ((), ())),
                               preferred_element_type=jnp.float32)


def _softmax_pv(s, vh):
    m = jnp.max(s, axis=-1, keepdims=True)
    p = jnp.exp(s - m)
    l = jnp.sum(p, axis=-1, keepdims=True)
    o = jnp.dot(p.astype(jnp.bfloat16), vh, preferred_element_type=jnp.float32)
    r = pl.reciprocal(l, approx=True)
    r = r * (2.0 - l * r)
    return (o * r).astype(jnp.bfloat16)


def _kernel(ax, ak, av, awq, awo, bx, bk, bv, bwq, bwo, o_hbm,
            acc, kvbuf, xbuf, wqbuf, wobuf, qbuf, obuf, kvsem, xsem, wsem, osem):
    scale = DH ** -0.5
    t = pl.program_id(0)
    total = pl.num_programs(0)
    ng = qbuf.shape[1]
    nj = total // ng
    sq = acc.shape[1]
    d_model = xbuf.shape[2]
    g = t // nj
    j = t % nj
    kv_hbm = (ak, av, bk, bv)
    x_hbm = (ax, bx)
    wq_hbm = (awq, bwq)
    wo_hbm = (awo, bwo)
    w = HG * DH

    def kv_copy(tt, i):
        tj = tt % nj
        tg = tt // nj
        st = tt % RING
        return pltpu.make_async_copy(
            kv_hbm[i].at[pl.ds(tj * NB, NB), pl.ds(tg * HG, HG)],
            kvbuf.at[st, i], kvsem.at[st, i])

    def wq_copy(br, gg):
        return pltpu.make_async_copy(
            wq_hbm[br].at[:, pl.ds(gg * w, w)], wqbuf.at[br, gg], wsem.at[0, br, gg])

    def wo_copy(br, gg):
        return pltpu.make_async_copy(
            wo_hbm[br].at[pl.ds(gg * w, w), :], wobuf.at[br, gg], wsem.at[1, br, gg])

    def out_copy(b):
        return pltpu.make_async_copy(obuf.at[b], o_hbm.at[b], osem.at[b])

    @pl.when(t == 0)
    def _():
        mh = xbuf.shape[1] // 2

        def xa_copy(hf):
            return pltpu.make_async_copy(
                x_hbm[0].at[pl.ds(hf * mh, mh)], xbuf.at[0, pl.ds(hf * mh, mh)],
                xsem.at[2 * hf])

        def xb_copy():
            return pltpu.make_async_copy(x_hbm[1], xbuf.at[1], xsem.at[1])

        def qproj(br, gg):
            q = jnp.dot(xbuf[br], wqbuf[br, gg], preferred_element_type=jnp.float32)
            qbuf[br, gg] = (q * scale).astype(jnp.bfloat16)

        xa_copy(0).start()
        wq_copy(0, 0).start()
        xa_copy(1).start()
        acc[...] = jnp.zeros(acc.shape, acc.dtype)
        xa_copy(0).wait()
        wq_copy(0, 0).wait()
        xb_copy().start()
        wq_copy(1, 0).start()
        wq_copy(0, 1).start()
        for hf in range(2):
            if hf == 1:
                xa_copy(1).wait()
            q = jnp.dot(xbuf[0, pl.ds(hf * mh, mh)], wqbuf[0, 0],
                        preferred_element_type=jnp.float32)
            qbuf[0, 0, pl.ds(hf * mh, mh)] = (q * scale).astype(jnp.bfloat16)

        def body(gg, carry):
            @pl.when(gg == 0)
            def _():
                xb_copy().wait()
            wq_copy(1, gg).wait()
            wq_copy(0, gg + 1).wait()

            @pl.when(gg == 0)
            def _():
                wq_copy(1, 1).start()
                for g2 in range(2, ng):
                    wq_copy(0, g2).start()
                    wq_copy(1, g2).start()

            @pl.when(jnp.logical_and(gg >= LAG, gg - LAG < RING - 1))
            def _():
                for i in range(4):
                    kv_copy(gg - LAG, i).start()

            @pl.when(gg >= LAG)
            def _():
                wo_copy(0, gg - LAG).start()
                wo_copy(1, gg - LAG).start()

            qproj(1, gg)
            qproj(0, gg + 1)
            return carry

        jax.lax.fori_loop(0, ng - 1, body, 0)
        wq_copy(1, ng - 1).wait()
        qproj(1, ng - 1)
        for d in range(ng - 1 - LAG, RING - 1):
            for i in range(4):
                kv_copy(d, i).start()
        for gg in range(ng - 1 - LAG, ng):
            wo_copy(0, gg).start()
            wo_copy(1, gg).start()

    @pl.when(t + RING - 1 < total)
    def _():
        for i in range(4):
            kv_copy(t + RING - 1, i).start()

    @pl.when(j == 0)
    def _():
        wo_copy(0, g).wait()
        wo_copy(1, g).wait()

    for i in range(4):
        kv_copy(t, i).wait()
    cur = t % RING

    def attend(last):
        units = [(s, br, h) for s in range(NB) for br in range(2) for h in range(HG)]
        n = len(units)
        scores = {}

        def issue(i):
            s, br, h = units[i]
            r0 = pl.multiple_of((j * NB + s) * sq, 32)
            qh = qbuf[br, g, pl.ds(r0, sq), h * DH:(h + 1) * DH]
            scores[i] = _qk(qh, kvbuf[cur, 2 * br, s, h])

        issue(0)
        outs = []
        for i in range(n):
            if i + 1 < n:
                issue(i + 1)
            s, br, h = units[i]
            outs.append(_softmax_pv(scores.pop(i), kvbuf[cur, 2 * br + 1, s, h]))
            if h == HG - 1:
                b = j * NB + s
                cols = slice(br * d_model, (br + 1) * d_model)
                o = jnp.concatenate(outs, axis=-1)
                outs = []
                r = jnp.dot(o, wobuf[br, g], preferred_element_type=jnp.float32)
                if not last:
                    acc[b, :, cols] += r
                else:
                    obuf[b, :, cols] = (acc[b, :, cols] + r).astype(obuf.dtype)
                    if br == 1:
                        out_copy(b).start()

    @pl.when(g < ng - 1)
    def _():
        attend(False)

    @pl.when(g == ng - 1)
    def _():
        attend(True)

    @pl.when(t == total - 1)
    def _():
        for b in range(nj * NB):
            out_copy(b).wait()


@jax.jit
def pallas_concat_heads__mha_block_cached__mha_block_cached__near_ridge_kernel(
    A_x: jax.Array,
    A_k_cache: jax.Array,
    A_v_cache: jax.Array,
    A_wq: jax.Array,
    A_wo: jax.Array,
    B_x: jax.Array,
    B_k_cache: jax.Array,
    B_v_cache: jax.Array,
    B_wq: jax.Array,
    B_wo: jax.Array,
):
    B, Sq, D = A_x.shape
    _, H, Sk, Dh = A_k_cache.shape
    ng = H // HG
    nj = B // NB
    anyspec = pl.BlockSpec(memory_space=pl.ANY)
    return pl.pallas_call(
        _kernel,
        grid=(ng * nj,),
        in_specs=[anyspec] * 10,
        out_specs=anyspec,
        out_shape=jax.ShapeDtypeStruct((B, Sq, 2 * D), jnp.bfloat16),
        scratch_shapes=[
            pltpu.VMEM((B, Sq, 2 * D), jnp.float32),
            pltpu.VMEM((RING, 4, NB, HG, Sk, Dh), jnp.bfloat16),
            pltpu.VMEM((2, B * Sq, D), jnp.bfloat16),
            pltpu.VMEM((2, ng, D, HG * Dh), jnp.bfloat16),
            pltpu.VMEM((2, ng, HG * Dh, D), jnp.bfloat16),
            pltpu.VMEM((2, ng, B * Sq, HG * Dh), jnp.bfloat16),
            pltpu.VMEM((B, Sq, 2 * D), jnp.bfloat16),
            pltpu.SemaphoreType.DMA((RING, 4)),
            pltpu.SemaphoreType.DMA((3,)),
            pltpu.SemaphoreType.DMA((2, 2, ng)),
            pltpu.SemaphoreType.DMA((B,)),
        ],
        compiler_params=pltpu.CompilerParams(
            dimension_semantics=("arbitrary",),
            disable_bounds_checks=True,
            vmem_limit_bytes=120 * 1024 * 1024),
    )(A_x.reshape(B * Sq, D), A_k_cache, A_v_cache, A_wq, A_wo,
      B_x.reshape(B * Sq, D), B_k_cache, B_v_cache, B_wq, B_wo)
```
